```python
import os as _os
_os.environ.setdefault("JAX_PLATFORMS", "cpu")
import jax
import jax.numpy as jnp

def _softmax(x, axis=-1):
    return jax.nn.softmax(x, axis=axis)
def _gelu(x):
    return jax.nn.gelu(x, approximate=True)
def _silu(x):
    return jax.nn.silu(x)
def _sigmoid(x):
    return jax.nn.sigmoid(x)
def _layernorm(x, axis=-1, eps=1e-5):
    m = jnp.mean(x, axis=axis, keepdims=True)
    v = jnp.var(x, axis=axis, keepdims=True)
    return (x - m) / jnp.sqrt(v + eps)
def _scatter_add(tgt, idx, src, axis=0):
    return tgt.at[idx].add(src)
def _segment_sum(src, seg, n):
    return jax.ops.segment_sum(src, seg, n)
class _Rng:
    def __init__(self, key):
        self._k = key
    def _next(self):
        self._k, sub = jax.random.split(self._k)
        return sub
    def normal(self, shape):
        return jax.random.normal(self._next(), shape, dtype=jnp.bfloat16)
    def randint(self, lo, hi, shape):
        return jax.random.randint(self._next(), shape, lo, hi, dtype=jnp.int32)
    def uniform(self, shape, lo=0.0, hi=1.0):
        return jax.random.uniform(self._next(), shape, jnp.bfloat16, lo, hi)
    def permutation(self, n):
        return jax.random.permutation(self._next(), n)


kernel_name = 'sequential_preLN__mha_block__moe_arch_mod__prompt'

def setup_inputs():
    _rng = _Rng(jax.random.key(int.from_bytes(__import__("os").urandom(4), "little")))
    _w = (lambda a: (lambda t: t.astype(jnp.bfloat16) if jnp.issubdtype(t.dtype, jnp.floating) else t)(jnp.asarray(a)))
    def _A_setup():
        B, S, D, H = 1, 2048, 640, 32
        return {
            "x": _w((lambda *s: _rng.normal(s) * 0.05)(B, S, D)),
            "wqkv": _w((lambda *s: _rng.normal(s) * 0.05)(D, 3 * D)),
            "wo": _w((lambda *s: _rng.normal(s) * 0.05)(D, D)),
        }
    _A_in = _A_setup()

    def _B_setup():
        B, S, D, F, C = 1, 2048, 640, 1536, 1
        return {
            "x": _w((lambda *s: _rng.normal(s) * 0.05)(B, S, D)),
            "w_r": _w((lambda *s: _rng.normal(s) * 0.05)(D)),
            "w_gate": _w((lambda *s: _rng.normal(s) * 0.05)(D, F)),
            "w_up": _w((lambda *s: _rng.normal(s) * 0.05)(D, F)),
            "w_down": _w((lambda *s: _rng.normal(s) * 0.05)(F, D)),
        }
    _B_in = _B_setup()

    return {
        "A_x": _A_in["x"],
        "A_wqkv": _A_in["wqkv"],
        "A_wo": _A_in["wo"],
        "B_x": _B_in["x"],
        "B_w_r": _B_in["w_r"],
        "B_w_gate": _B_in["w_gate"],
        "B_w_up": _B_in["w_up"],
        "B_w_down": _B_in["w_down"],
    }

def reference(A_x, A_wqkv, A_wo, B_x, B_w_r, B_w_gate, B_w_up, B_w_down):
    def _A_ref(x, wqkv, wo):
        B, S, D = x.shape
        H = 32
        Dh = D // H
        qkv = (lambda x, *d: x.transpose(*d))((x @ wqkv).reshape(B, S, 3, H, Dh), 2, 0, 3, 1, 4)
        q, k, v = qkv[0], qkv[1], qkv[2]
        scores = jnp.einsum("bhqd,bhkd->bhqk", q, k) * (Dh ** -0.5)
        p = _softmax(scores, axis=-1)
        o = jnp.einsum("bhqk,bhkd->bhqd", p, v)
        return (lambda x, *d: x.transpose(*d))(o, 0, 2, 1, 3).reshape(B, S, D) @ wo

    def _B_ref(x, w_r, w_gate, w_up, w_down):
        B, S, D = x.shape
        C = 1
        r = x @ w_r
        idx = jnp.argsort(-r, axis=-1)[:, :C]
        idx_e = jnp.repeat(idx.reshape(B, C, 1), D, axis=2)
        x_sel = jnp.take_along_axis(x, idx_e, axis=1)
        g = _silu(x_sel @ w_gate)
        u = x_sel @ w_up
        y = (g * u) @ w_down
        r_sel = _sigmoid(jnp.take_along_axis(r, idx, axis=1))
        y = y * r_sel.reshape(B, C, 1)
        b_off = (jnp.arange(B) * S).reshape(B, 1)
        flat_idx = (idx + b_off).reshape(B * C)
        zero = (x * 0.0).reshape(B * S, D)
        upd = _scatter_add(zero, flat_idx, y.reshape(B * C, D), axis=0)
        return x + upd.reshape(B, S, D)

    x = A_x
    h = x + _A_ref(_layernorm(x, axis=-1), A_wqkv, A_wo)
    h2 = h + _B_ref(_layernorm(h, axis=-1), B_w_r, B_w_gate, B_w_up, B_w_down)
    return h2
```

```python
import functools

import jax
import jax.numpy as jnp
import jax.experimental.pallas as pl
import jax.experimental.pallas.tpu as pltpu

S = 2048
D = 640
H = 32
DH = 20
F = 1536
HPG = 6
NG = 6
SLOT = 32
TQ = 256
NQ = S // TQ
EPS = 1e-5
LOG2E = 1.4426950408889634


def _layernorm(x):
    m = jnp.mean(x, axis=-1, keepdims=True)
    xc = x - m
    v = jnp.mean(xc * xc, axis=-1, keepdims=True)
    return xc * jax.lax.rsqrt(v + EPS)


def _pad_groups(w):
    parts = []
    for g in range(NG):
        lo = g * HPG * DH
        hi = min(lo + HPG * DH, D)
        parts.append(w[:, lo:hi])
        parts.append(jnp.zeros((w.shape[0], 128 - (hi - lo)), w.dtype))
    return jnp.concatenate(parts, axis=1)


def _kernel(x_ref, wqkv_ref, wo_ref, wr_ref, wg_hbm, wu_hbm, wd_hbm,
            o_ref,
            k_scr, qt_scr, vt_scr, wo_scr, ot_scr, ln2_scr, r_scr,
            wg_scr, wu_scr, wd_scr, sems):
    qi = pl.program_id(0)
    f32 = jnp.float32
    bf16 = jnp.bfloat16

    @pl.when(qi == 0)
    def _prologue():
        pltpu.make_async_copy(wg_hbm, wg_scr, sems.at[0]).start()
        pltpu.make_async_copy(wu_hbm, wu_scr, sems.at[1]).start()
        pltpu.make_async_copy(wd_hbm, wd_scr, sems.at[2]).start()

        ln = _layernorm(x_ref[...].astype(f32)).astype(bf16)
        wq = _pad_groups(wqkv_ref[:, 0:D].astype(f32)).astype(bf16)
        wk = _pad_groups(wqkv_ref[:, D:2 * D].astype(f32)).astype(bf16)
        wv = wqkv_ref[:, 2 * D:3 * D]
        k = jnp.dot(ln, wk, preferred_element_type=f32).astype(bf16)
        for g in range(NG):
            k_scr[g] = k[:, g * 128:(g + 1) * 128]
        q = jnp.dot(ln, wq, preferred_element_type=f32) * (DH ** -0.5 * LOG2E)
        qt = q.T.astype(bf16)
        for t in range(NQ):
            qt_scr[t] = qt[:, t * TQ:(t + 1) * TQ]
        vt = jnp.dot(ln, wv, preferred_element_type=f32).T
        wo = wo_ref[...].astype(f32)
        ones = jnp.ones((1, S), f32)
        zv = jnp.zeros((SLOT - DH - 1, S), f32)
        zw = jnp.zeros((SLOT - DH, D), f32)
        for h in range(H):
            blk = jnp.concatenate([vt[h * DH:(h + 1) * DH], ones, zv], axis=0)
            vt_scr[h] = blk.astype(bf16)
            wblk = jnp.concatenate([wo[h * DH:(h + 1) * DH], zw], axis=0)
            wo_scr[h * SLOT:(h + 1) * SLOT, :] = wblk.astype(bf16)

    row = jax.lax.broadcasted_iota(jnp.int32, (128, TQ), 0)

    def head(h, carry):
        g = h // HPG
        lo = (h - g * HPG) * DH
        qg = qt_scr[qi, pl.ds(pl.multiple_of(g * 128, 128), 128), :]
        qm = jnp.where((row >= lo) & (row < lo + DH), qg, jnp.zeros_like(qg))
        st = jnp.dot(k_scr[g], qm, preferred_element_type=f32)
        m = jnp.max(st, axis=0, keepdims=True)
        p = jnp.exp2(st - m).astype(bf16)
        ot = jnp.dot(vt_scr[h], p, preferred_element_type=f32)
        ot = ot * (1.0 / ot[DH:DH + 1, :])
        ot_scr[pl.ds(pl.multiple_of(h * SLOT, SLOT), SLOT), :] = ot
        return carry

    jax.lax.fori_loop(0, H, head, 0)

    o = ot_scr[...].T.astype(bf16)
    attn = jnp.dot(o, wo_scr[...], preferred_element_type=f32)
    r0 = pl.multiple_of(qi * TQ, TQ)
    hres = x_ref[pl.ds(r0, TQ), :].astype(f32) + attn
    ln2 = _layernorm(hres)
    ln2_scr[pl.ds(r0, TQ), :] = ln2
    r_scr[pl.ds(r0, TQ), :] = jnp.sum(ln2 * wr_ref[...].astype(f32), axis=-1, keepdims=True)
    o_ref[pl.ds(r0, TQ), :] = (hres + ln2).astype(o_ref.dtype)

    @pl.when(qi == NQ - 1)
    def _epilogue():
        pltpu.make_async_copy(wg_hbm, wg_scr, sems.at[0]).wait()
        pltpu.make_async_copy(wu_hbm, wu_scr, sems.at[1]).wait()
        pltpu.make_async_copy(wd_hbm, wd_scr, sems.at[2]).wait()
        r = r_scr[...]
        rmax = jnp.max(r)
        ids = jax.lax.broadcasted_iota(jnp.int32, (S, 1), 0)
        idx = jnp.min(jnp.where(r >= rmax, ids, S))
        xs = jnp.broadcast_to(ln2_scr[pl.ds(idx, 1), :], (8, D)).astype(bf16)
        a = jnp.dot(xs, wg_scr[...], preferred_element_type=f32)
        u = jnp.dot(xs, wu_scr[...], preferred_element_type=f32)
        gu = (a * jax.nn.sigmoid(a) * u).astype(bf16)
        y = jnp.dot(gu, wd_scr[...], preferred_element_type=f32)[0:1, :]
        y = y * jax.nn.sigmoid(jnp.full((1, D), rmax, f32))
        base = pl.multiple_of((idx // 16) * 16, 16)
        rr = jax.lax.broadcasted_iota(jnp.int32, (16, D), 0)
        cur = o_ref[pl.ds(base, 16), :].astype(f32)
        o_ref[pl.ds(base, 16), :] = (
            cur + jnp.where(rr == idx - base, y, 0.0)).astype(o_ref.dtype)


@jax.jit
def pallas_sequential_preLN__mha_block__moe_arch_mod__prompt_kernel(
    A_x: jax.Array,
    A_wqkv: jax.Array,
    A_wo: jax.Array,
    B_x: jax.Array,
    B_w_r: jax.Array,
    B_w_gate: jax.Array,
    B_w_up: jax.Array,
    B_w_down: jax.Array,
):
    x = A_x.reshape(S, D)
    wr = B_w_r.reshape(1, D)
    full = lambda shape: pl.BlockSpec(shape, lambda i: (0,) * len(shape))
    out = pl.pallas_call(
        _kernel,
        grid=(NQ,),
        in_specs=[
            full((S, D)), full((D, 3 * D)), full((D, D)), full((1, D)),
            pl.BlockSpec(memory_space=pl.ANY),
            pl.BlockSpec(memory_space=pl.ANY),
            pl.BlockSpec(memory_space=pl.ANY),
        ],
        out_specs=full((S, D)),
        out_shape=jax.ShapeDtypeStruct((S, D), A_x.dtype),
        scratch_shapes=[
            pltpu.VMEM((NG, S, 128), jnp.bfloat16),
            pltpu.VMEM((NQ, NG * 128, TQ), jnp.bfloat16),
            pltpu.VMEM((H, SLOT, S), jnp.bfloat16),
            pltpu.VMEM((H * SLOT, D), jnp.bfloat16),
            pltpu.VMEM((H * SLOT, TQ), jnp.float32),
            pltpu.VMEM((S, D), jnp.float32),
            pltpu.VMEM((S, 1), jnp.float32),
            pltpu.VMEM((D, F), jnp.bfloat16),
            pltpu.VMEM((D, F), jnp.bfloat16),
            pltpu.VMEM((F, D), jnp.bfloat16),
            pltpu.SemaphoreType.DMA((3,)),
        ],
        compiler_params=pltpu.CompilerParams(
            dimension_semantics=("arbitrary",),
            vmem_limit_bytes=100 * 1024 * 1024,
        ),
    )(x, A_wqkv, A_wo, wr, B_w_gate, B_w_up, B_w_down)
    return out.reshape(1, S, D)
```

```python
import functools

import jax
import jax.numpy as jnp
import jax.experimental.pallas as pl
import jax.experimental.pallas.tpu as pltpu

S = 2048
D = 640
H = 32
DH = 20
F = 1536
HPG = 6
NG = 6
SLOT = 32
TQ = 512
NQ = S // TQ
EPS = 1e-5
KC = 128
LOG2E = 1.4426950408889634


def _layernorm(x):
    m = jnp.mean(x, axis=-1, keepdims=True)
    xc = x - m
    v = jnp.mean(xc * xc, axis=-1, keepdims=True)
    return xc * jax.lax.rsqrt(v + EPS)


def _pad_groups(w):
    parts = []
    for g in range(NG):
        lo = g * HPG * DH
        hi = min(lo + HPG * DH, D)
        parts.append(w[:, lo:hi])
        parts.append(jnp.zeros((w.shape[0], 128 - (hi - lo)), w.dtype))
    return jnp.concatenate(parts, axis=1)


def _kernel(x_ref, wqkv_ref, wo_ref, wr_ref, wg_hbm, wu_hbm, wd_hbm,
            o_ref,
            k_scr, qt_scr, vt_scr, wo_scr, ot_scr, ln2_scr, r_scr,
            wg_scr, wu_scr, wd_scr, sa_scr, sb_scr, sems):
    qi = pl.program_id(0)
    f32 = jnp.float32
    bf16 = jnp.bfloat16

    @pl.when(qi == 0)
    def _prologue():
        pltpu.make_async_copy(wg_hbm, wg_scr, sems.at[0]).start()
        pltpu.make_async_copy(wu_hbm, wu_scr, sems.at[1]).start()
        pltpu.make_async_copy(wd_hbm, wd_scr, sems.at[2]).start()

        ln = _layernorm(x_ref[...].astype(f32)).astype(bf16)
        wq = _pad_groups(wqkv_ref[:, 0:D].astype(f32)).T.astype(bf16)
        wk = _pad_groups(wqkv_ref[:, D:2 * D].astype(f32)).astype(bf16)
        wv = wqkv_ref[:, 2 * D:3 * D].astype(f32).T.astype(bf16)
        k = jnp.dot(ln, wk, preferred_element_type=f32).astype(bf16)
        for g in range(NG):
            k_scr[g] = k[:, g * 128:(g + 1) * 128]
        nt = (((1,), (1,)), ((), ()))
        qt = (jax.lax.dot_general(wq, ln, nt, preferred_element_type=f32)
              * (DH ** -0.5 * LOG2E)).astype(bf16)
        for t in range(NQ):
            qt_scr[t] = qt[:, t * TQ:(t + 1) * TQ]
        vt = jax.lax.dot_general(wv, ln, nt, preferred_element_type=f32)
        wo = wo_ref[...].astype(f32)
        ones = jnp.ones((1, S), f32)
        zv = jnp.zeros((SLOT - DH - 1, S), f32)
        zw = jnp.zeros((SLOT - DH, D), f32)
        for h in range(H):
            blk = jnp.concatenate([vt[h * DH:(h + 1) * DH], ones, zv], axis=0)
            vt_scr[h] = blk.astype(bf16)
            wblk = jnp.concatenate([wo[h * DH:(h + 1) * DH], zw], axis=0)
            wo_scr[h * SLOT:(h + 1) * SLOT, :] = wblk.astype(bf16)

    row = jax.lax.broadcasted_iota(jnp.int32, (128, TQ), 0)

    def qmask(h):
        g = h // HPG
        lo = (h - g * HPG) * DH
        qg = qt_scr[qi, pl.ds(pl.multiple_of(g * 128, 128), 128), :]
        return g, jnp.where((row >= lo) & (row < lo + DH), qg, jnp.zeros_like(qg))

    def fused(hq, sq_ref, hp, sp_ref, mp):
        g, qm = qmask(hq)
        macc = None
        acc = None
        for c in range(S // KC):
            ks = slice(c * KC, (c + 1) * KC)
            st = jnp.dot(k_scr[g, ks, :], qm, preferred_element_type=f32)
            sq_ref[ks, :] = st
            mc = jnp.max(st, axis=0, keepdims=True)
            macc = mc if macc is None else jnp.maximum(macc, mc)
            if hp is not None:
                p = jnp.exp2(sp_ref[ks, :] - mp).astype(bf16)
                oc = jnp.dot(vt_scr[hp, :, ks], p, preferred_element_type=f32)
                acc = oc if acc is None else acc + oc
        if hp is not None:
            acc = acc * (1.0 / acc[DH:DH + 1, :])
            ot_scr[pl.ds(pl.multiple_of(hp * SLOT, SLOT), SLOT), :] = acc
        return macc

    def pair(i, ma):
        h = 2 * i
        mb = fused(h + 1, sb_scr, h, sa_scr, ma)
        return fused(jnp.minimum(h + 2, H - 1), sa_scr, h + 1, sb_scr, mb)

    jax.lax.fori_loop(0, H // 2, pair, fused(0, sa_scr, None, None, None))

    o = ot_scr[...].T.astype(bf16)
    attn = jnp.dot(o, wo_scr[...], preferred_element_type=f32)
    r0 = pl.multiple_of(qi * TQ, TQ)
    hres = x_ref[pl.ds(r0, TQ), :].astype(f32) + attn
    ln2 = _layernorm(hres)
    ln2_scr[pl.ds(r0, TQ), :] = ln2
    r_scr[pl.ds(r0, TQ), :] = jnp.sum(ln2 * wr_ref[...].astype(f32), axis=-1, keepdims=True)
    o_ref[pl.ds(r0, TQ), :] = (hres + ln2).astype(o_ref.dtype)

    @pl.when(qi == NQ - 1)
    def _epilogue():
        pltpu.make_async_copy(wg_hbm, wg_scr, sems.at[0]).wait()
        pltpu.make_async_copy(wu_hbm, wu_scr, sems.at[1]).wait()
        pltpu.make_async_copy(wd_hbm, wd_scr, sems.at[2]).wait()
        r = r_scr[...]
        rmax = jnp.max(r)
        ids = jax.lax.broadcasted_iota(jnp.int32, (S, 1), 0)
        idx = jnp.min(jnp.where(r >= rmax, ids, S))
        xs = jnp.broadcast_to(ln2_scr[pl.ds(idx, 1), :], (8, D)).astype(bf16)
        a = jnp.dot(xs, wg_scr[...], preferred_element_type=f32)
        u = jnp.dot(xs, wu_scr[...], preferred_element_type=f32)
        gu = (a * jax.nn.sigmoid(a) * u).astype(bf16)
        y = jnp.dot(gu, wd_scr[...], preferred_element_type=f32)[0:1, :]
        y = y * jax.nn.sigmoid(jnp.full((1, D), rmax, f32))
        base = pl.multiple_of((idx // 16) * 16, 16)
        rr = jax.lax.broadcasted_iota(jnp.int32, (16, D), 0)
        cur = o_ref[pl.ds(base, 16), :].astype(f32)
        o_ref[pl.ds(base, 16), :] = (
            cur + jnp.where(rr == idx - base, y, 0.0)).astype(o_ref.dtype)


@jax.jit
def pallas_sequential_preLN__mha_block__moe_arch_mod__prompt_kernel(
    A_x: jax.Array,
    A_wqkv: jax.Array,
    A_wo: jax.Array,
    B_x: jax.Array,
    B_w_r: jax.Array,
    B_w_gate: jax.Array,
    B_w_up: jax.Array,
    B_w_down: jax.Array,
):
    x = A_x.reshape(S, D)
    wr = B_w_r.reshape(1, D)
    full = lambda shape: pl.BlockSpec(shape, lambda i: (0,) * len(shape))
    out = pl.pallas_call(
        _kernel,
        grid=(NQ,),
        in_specs=[
            full((S, D)), full((D, 3 * D)), full((D, D)), full((1, D)),
            pl.BlockSpec(memory_space=pl.ANY),
            pl.BlockSpec(memory_space=pl.ANY),
            pl.BlockSpec(memory_space=pl.ANY),
        ],
        out_specs=full((S, D)),
        out_shape=jax.ShapeDtypeStruct((S, D), A_x.dtype),
        scratch_shapes=[
            pltpu.VMEM((NG, S, 128), jnp.bfloat16),
            pltpu.VMEM((NQ, NG * 128, TQ), jnp.bfloat16),
            pltpu.VMEM((H, SLOT, S), jnp.bfloat16),
            pltpu.VMEM((H * SLOT, D), jnp.bfloat16),
            pltpu.VMEM((H * SLOT, TQ), jnp.float32),
            pltpu.VMEM((S, D), jnp.float32),
            pltpu.VMEM((S, 1), jnp.float32),
            pltpu.VMEM((D, F), jnp.bfloat16),
            pltpu.VMEM((D, F), jnp.bfloat16),
            pltpu.VMEM((F, D), jnp.bfloat16),
            pltpu.VMEM((S, TQ), jnp.float32),
            pltpu.VMEM((S, TQ), jnp.float32),
            pltpu.SemaphoreType.DMA((3,)),
        ],
        compiler_params=pltpu.CompilerParams(
            dimension_semantics=("arbitrary",),
            vmem_limit_bytes=100 * 1024 * 1024,
        ),
    )(x, A_wqkv, A_wo, wr, B_w_gate, B_w_up, B_w_down)
    return out.reshape(1, S, D)
```
